```python
import os as _os
_os.environ.setdefault("JAX_PLATFORMS", "cpu")
import jax
import jax.numpy as jnp

def _softmax(x, axis=-1):
    return jax.nn.softmax(x, axis=axis)
def _gelu(x):
    return jax.nn.gelu(x, approximate=True)
def _silu(x):
    return jax.nn.silu(x)
def _sigmoid(x):
    return jax.nn.sigmoid(x)
def _layernorm(x, axis=-1, eps=1e-5):
    m = jnp.mean(x, axis=axis, keepdims=True)
    v = jnp.var(x, axis=axis, keepdims=True)
    return (x - m) / jnp.sqrt(v + eps)
def _scatter_add(tgt, idx, src, axis=0):
    return tgt.at[idx].add(src)
def _segment_sum(src, seg, n):
    return jax.ops.segment_sum(src, seg, n)
class _Rng:
    def __init__(self, key):
        self._k = key
    def _next(self):
        self._k, sub = jax.random.split(self._k)
        return sub
    def normal(self, shape):
        return jax.random.normal(self._next(), shape, dtype=jnp.bfloat16)
    def randint(self, lo, hi, shape):
        return jax.random.randint(self._next(), shape, lo, hi, dtype=jnp.int32)
    def uniform(self, shape, lo=0.0, hi=1.0):
        return jax.random.uniform(self._next(), shape, jnp.bfloat16, lo, hi)
    def permutation(self, n):
        return jax.random.permutation(self._next(), n)


kernel_name = 'concat_heads__linear_attn_block__sliding_local_dilated__prompt'

def setup_inputs():
    _rng = _Rng(jax.random.key(int.from_bytes(__import__("os").urandom(4), "little")))
    _w = (lambda a: (lambda t: t.astype(jnp.bfloat16) if jnp.issubdtype(t.dtype, jnp.floating) else t)(jnp.asarray(a)))
    def _A_setup():
        B, S, D = 1, 2048, 576
        return {
            "x": _w((lambda *s: _rng.normal(s) * 0.05)(B, S, D)),
            "wqkv": _w((lambda *s: _rng.normal(s) * 1.6)(D, 3 * D)),
            "wo": _w((lambda *s: _rng.normal(s) * 0.4)(D, D)),
        }
    _A_in = _A_setup()

    def _B_setup():
        B, S, D = 1, 2048, 576
        return {
            "x": _w((lambda *s: _rng.normal(s) * 0.2)(B, S, D)),
            "wqkv": _w((lambda *s: _rng.normal(s) * 0.2)(D, 3 * D)),
            "wo": _w((lambda *s: _rng.normal(s) * 0.05)(D, D)),
        }
    _B_in = _B_setup()

    return {
        "A_x": _A_in["x"],
        "A_wqkv": _A_in["wqkv"],
        "A_wo": _A_in["wo"],
        "B_x": _B_in["x"],
        "B_wqkv": _B_in["wqkv"],
        "B_wo": _B_in["wo"],
    }

def reference(A_x, A_wqkv, A_wo, B_x, B_wqkv, B_wo):
    def _A_ref(x, wqkv, wo):
        B, S, D = x.shape
        H = 32; Dh = D // H
        qkv = (lambda x, *d: x.transpose(*d))((x @ wqkv).reshape(B, S, 3, H, Dh), 2, 0, 3, 1, 4)
        q, k, v = qkv[0], qkv[1], qkv[2]
        phi = lambda t: jnp.where(t > 0, t + 1, jnp.exp(t)) + 1e-6
        pq, pk = phi(q), phi(k)
        kv = jnp.einsum("bhsd,bhse->bhde", pk, v)
        z = jnp.einsum("bhsd->bhd", pk)
        num = jnp.einsum("bhqd,bhde->bhqe", pq, kv)
        den = jnp.einsum("bhqd,bhd->bhq", pq, z)[..., None] + 1e-6
        o = num / den
        return (lambda x, *d: x.transpose(*d))(o, 0, 2, 1, 3).reshape(B, S, D) @ wo

    def _B_ref(x, wqkv, wo):
        B, S, D = x.shape
        H = 32; Dh = D // H
        W, dil = 8, 2
        qkv = (lambda x, *d: x.transpose(*d))((x @ wqkv).reshape(B, S, 3, H, Dh), 2, 0, 3, 1, 4)
        q, k, v = qkv[0], qkv[1], qkv[2]
        scale = Dh ** -0.5
        pos = jnp.arange(S)
        off = jnp.arange(W) * dil
        idx = pos[:, None] - off[None, :]
        mask = idx >= 0
        idx_c = jnp.where(mask, idx, 0).reshape(-1)
        kg = k[:, :, idx_c, :].reshape(B, H, S, W, Dh)
        vg = v[:, :, idx_c, :].reshape(B, H, S, W, Dh)
        logits = jnp.einsum("bhsd,bhswd->bhsw", q, kg) * scale
        logits = jnp.where(mask[None, None, :, :], logits, -1e9)
        attn = _softmax(logits, axis=-1)
        o = jnp.einsum("bhsw,bhswd->bhsd", attn, vg)
        return (lambda x, *d: x.transpose(*d))(o, 0, 2, 1, 3).reshape(B, S, D) @ wo

    a = _A_ref(A_x, A_wqkv, A_wo)
    b = _B_ref(B_x, B_wqkv, B_wo)
    return jnp.concatenate([a, b], axis=-1)
```

```python
import jax
import jax.numpy as jnp
import numpy as np
from jax import lax
import jax.experimental.pallas as pl
import jax.experimental.pallas.tpu as pltpu

S = 2048
D = 576
H = 32
DH = 18
DP = 640
WIN = 8
DIL = 2
HALO = 16
T = 256
T1 = 256
SUB = 16
NB = S // T
F32 = jnp.float32
BF16 = jnp.bfloat16
U32 = jnp.uint32
NN = (((1,), (0,)), ((), ()))
NT = (((1,), (1,)), ((), ()))


def _phi(t):
    return jnp.where(t > 0, t + 1.0, jnp.exp(t)) + 1e-6


def _dot(a, b, dims=NN):
    return lax.dot_general(a, b, dims, preferred_element_type=F32)


def _recip(d):
    r = pl.reciprocal(d, approx=True)
    return r * (2.0 - d * r)


def _ldw(ref, r0=None, r1=None, n=5):
    sl = slice(None) if r0 is None else slice(r0 // 2, r1 // 2)
    return pltpu.bitcast(jnp.concatenate([ref[j, sl, :] for j in range(n)], axis=1), BF16)


def _stw(ref, r0, val):
    u = pltpu.bitcast(val, U32)
    for j in range(val.shape[1] // 128):
        ref[j, r0 // 2:r0 // 2 + u.shape[0], :] = u[:, 128 * j:128 * j + 128]


def _kernel(xa_h, wa_h, woa_h, xb_h, wb_h, wob_h, out_h,
            xa_s, xb_s, wa_s, wb_s, woa_s, wob_s,
            ua, ub, uo, wk, wq, wb, wob, mt, g_s, zb, q0, q1, o0, o1, ostage,
            isem, osem):
    def cp(src, dst, k):
        return pltpu.make_async_copy(src, dst, isem.at[k])

    c_wak = cp(wa_h.at[:, 512:1152], wa_s.at[:, 512:1152], 0)
    c_xa0 = cp(xa_h.at[:, 0:T1], xa_s.at[:, 0:T1], 1)
    c_xa1 = cp(xa_h.at[:, T1:S], xa_s.at[:, T1:S], 2)
    c_waq = cp(wa_h.at[:, 0:512], wa_s.at[:, 0:512], 3)
    c_wav = cp(wa_h.at[:, 1152:1728], wa_s.at[:, 1152:1728], 4)
    c_wb = cp(wb_h, wb_s, 5)
    c_woa = cp(woa_h, woa_s, 6)
    c_wob = cp(wob_h, wob_s, 7)
    c_xb = cp(xb_h, xb_s, 8)
    c_wak.start()
    c_xa0.start()

    def transpose_chunks(w_s, u_s, chunks):
        for j in chunks:
            n = 128 if j < 13 else 64
            ct = w_s[:, 128 * j:128 * j + n].T
            ct = jnp.concatenate([ct, jnp.zeros((n, DP - D), BF16)], axis=1)
            _stw(u_s, 128 * j, ct)

    def perm_rows(u_s, base, dst, dst_row, dps=range(DH // 2)):
        for dp in dps:
            for kt in range(5):
                a = u_s[kt, pl.ds(base + dp, 16, stride=DH), :]
                b = u_s[kt, pl.ds(base + dp + DH // 2, 16, stride=DH), :]
                lo = (a & jnp.uint32(0xFFFF)) | (b << 16)
                hi = (a >> 16) | (b & jnp.uint32(0xFFFF0000))
                r0 = dst_row(2 * dp) // 2
                r1 = dst_row(2 * dp + 1) // 2
                dst[kt, r0:r0 + 16, :] = lo
                dst[kt, r1:r1 + 16, :] = hi

    c_wak.wait()
    transpose_chunks(wa_s, ua, range(4, 9))
    perm_rows(ua, 288, wk, lambda d: H * d)
    g_s[...] = jnp.zeros(g_s.shape, F32)

    def brow(p):
        def f(d):
            if d < 16:
                return (0, 512, 1152)[p] + H * d
            return (1024, 1088, 1664)[p] + H * (d - 16)
        return f

    def task_wob():
        w = wob_s[...]
        w = jnp.concatenate([jnp.zeros((D, 64), BF16), w], axis=1)
        _stw(uo, 0, w)
        perm_rows(uo, 0, wob, lambda d: H * d)
        for kt in range(5):
            wob[kt, D // 2:DP // 2, :] = jnp.zeros((32, 128), U32)

    def task_wb_pad():
        for kt in range(5):
            wb[kt, 864:896, :] = jnp.zeros((32, 128), U32)

    def nop():
        pass

    n1 = S // T1
    pre = {i: [] for i in range(n1 + 1)}
    mid = {i: [] for i in range(n1 + 1)}
    pre[0] += [c_xa0.wait, c_xa1.start, c_waq.start]
    pre[1] += [c_xa1.wait, c_wb.start, c_wav.start, c_woa.start, c_wob.start]
    pre[2] += [c_waq.wait, c_xb.start]
    mid[2] += [lambda: transpose_chunks(wa_s, ua, range(0, 4))]
    pre[3] += [c_wb.wait, lambda: perm_rows(ua, 0, wq, lambda d: H * d)]
    mid[3] += [lambda: transpose_chunks(wb_s, ub, range(0, 5))]
    pre[4] += [lambda: transpose_chunks(wb_s, ub, range(5, 10))]
    mid[4] += [lambda: transpose_chunks(wb_s, ub, range(10, 14)), task_wb_pad]
    pre[5] += [c_wav.wait, c_woa.wait, c_wob.wait, lambda: perm_rows(ub, 0, wb, brow(0))]
    mid[5] += [lambda: perm_rows(ub, 288, wb, brow(1))]
    pre[6] += [lambda: perm_rows(ub, 576, wb, brow(2))]
    mid[6] += [task_wob]
    pre[7] += [c_xb.wait]

    zero_rows = jnp.zeros((DP - D, T1), BF16)
    ones_rows = jnp.ones((DP - D, T1), BF16)
    for i in range(n1):
        for t in pre[i]:
            t()
        xt = xa_s[:, i * T1:(i + 1) * T1]
        kt_ = _dot(_ldw(wk), jnp.concatenate([xt, zero_rows], axis=0))
        pkt = _phi(kt_).astype(BF16)
        for t in mid[i]:
            t()
        g = _dot(pkt, jnp.concatenate([xt, ones_rows], axis=0), NT)
        g_s[...] += g

    def m_chain():
        mcs = []
        for c in range(4):
            gc = jnp.concatenate([g_s[H * d + 8 * c:H * d + 8 * c + 8, 0:D] for d in range(DH)], axis=0)
            n = 256 if c < 3 else 192
            cc = _dot(gc.astype(BF16), wa_s[:, 1152 + 128 * c:1152 + 128 * c + n])
            row = lax.broadcasted_iota(jnp.int32, (144, n), 0)
            col = lax.broadcasted_iota(jnp.int32, (144, n), 1) + 128 * c
            lo = ((row & 7) + 8 * c) * DH
            cc = jnp.where((col >= lo) & (col < lo + DH), cc, 0.0).astype(BF16)
            mcs.append(_dot(cc, woa_s[128 * c:128 * c + n, :]))
        mfull = jnp.concatenate([mcs[c][8 * d:8 * d + 8, :] for d in range(DH) for c in range(4)], axis=0)
        mT = mfull.astype(BF16).T
        mT = jnp.concatenate([mT, jnp.zeros((D, DP - D), BF16)], axis=1)
        _stw(mt, 0, mT)
        gt = g_s[:, 512:DP]
        lane576 = lax.broadcasted_iota(jnp.int32, (D, 128), 1)
        zb[...] = jnp.where(lane576 < 64, pltpu.roll(gt, 64, 1), gt)

    cscale = np.float32(DH ** -0.5 * np.log2(np.e))
    QT = (0, 1, 2, 3, 8)
    KT = (4, 5, 6, 7, 9)
    VT = (10, 11, 12, 13, 14)

    def proj_b(r0, qkv):
        xt = xb_s[:, pl.ds(r0, T)]
        xt = jnp.concatenate([xt, jnp.zeros((DP - D, T), BF16)], axis=0)
        x = xt.T
        body = pl.ds(HALO, T)
        r = _dot(x, _ldw(wb, 0, 512), NT)
        for j in range(4):
            qkv[j, body, :] = r[:, 128 * j:128 * j + 128] * cscale
        r = _dot(x, _ldw(wb, 512, 1152), NT)
        for j in range(4):
            qkv[4 + j, body, :] = r[:, 128 * j:128 * j + 128]
        tail = r[:, 512:640]
        lane = lax.broadcasted_iota(jnp.int32, (T, 128), 1)
        qkv[8, body, :] = jnp.where(lane < 64, tail * cscale, 0.0)
        qkv[9, body, :] = pltpu.roll(tail, 64, 1)
        r = _dot(x, _ldw(wb, 1152, 1792), NT)
        for j in range(5):
            qkv[10 + j, body, :] = r[:, 128 * j:128 * j + 128]

    def halo_first(qkv):
        for j in KT + VT:
            qkv[j, 0:HALO, :] = jnp.broadcast_to(qkv[j, HALO:HALO + 1, :], (HALO, 128))

    def halo_next(src, dst):
        for j in KT + VT:
            dst[j, 0:HALO, :] = src[j, T:T + HALO, :]

    def attn(r0, qkv, ob):
        for s in range(T // SUB):
            base = s * SUB
            q = [qkv[j, pl.ds(HALO + base, SUB), :] for j in QT]
            logits = []
            for w in range(WIN):
                sh = HALO - DIL * w
                acc = q[0] * qkv[KT[0], pl.ds(base + sh, SUB), :]
                for j in range(1, 5):
                    acc = acc + q[j] * qkv[KT[j], pl.ds(base + sh, SUB), :]
                acc = acc + pltpu.roll(acc, 64, 1)
                acc = acc + pltpu.roll(acc, 32, 1)
                if w > 0 and s == 0 and r0 is not None:
                    pos = lax.broadcasted_iota(jnp.int32, (SUB, 128), 0)
                    acc = jnp.where(pos >= DIL * w, acc, -1e9 * float(cscale))
                logits.append(acc)
            m = logits[0]
            for w in range(1, WIN):
                m = jnp.maximum(m, logits[w])
            es = [jnp.exp2(l - m) for l in logits]
            den = es[0]
            for w in range(1, WIN):
                den = den + es[w]
            inv = _recip(den)
            for j in range(5):
                acc = es[0] * qkv[VT[j], pl.ds(base + HALO, SUB), :]
                for w in range(1, WIN):
                    acc = acc + es[w] * qkv[VT[j], pl.ds(base + HALO - DIL * w, SUB), :]
                ob[j, pl.ds(s * SUB // 2, SUB // 2), :] = pltpu.bitcast((acc * inv).astype(BF16), U32)

    def out_block(i, r0, ob):
        rows = pl.ds(r0, T)
        xt = xa_s[:, pl.ds(r0, T)]
        xt = jnp.concatenate([xt, jnp.zeros((DP - D, T), BF16)], axis=0)
        qt = _dot(_ldw(wq), xt)
        pq = _phi(qt)
        z = zb[...]
        z = jnp.concatenate([z] * (T // 128), axis=1)
        pz = pq * z
        den = pz[0:H]
        for d in range(1, DH):
            den = den + pz[H * d:H * d + H]
        inv = _recip(den + 1e-6)
        pqs = jnp.concatenate([pq[H * d:H * d + H] * inv for d in range(DH)], axis=0).astype(BF16)
        pqs = jnp.concatenate([pqs, jnp.zeros((DP - D, T), BF16)], axis=0)
        rb = _dot(_ldw(ob), _ldw(wob)).astype(BF16)
        ostage[rows, D:640] = rb[:, 64:128]
        ostage[rows, 640:2 * D] = rb[:, 128:DP]
        oat = _dot(_ldw(mt), pqs)
        ostage[rows, 0:D] = oat.astype(BF16).T
        pltpu.make_async_copy(ostage.at[rows, :], out_h.at[rows, :], osem.at[i]).start()

    Q = (q0, q1)
    O = (o0, o1)

    proj_b(0, Q[0])
    halo_first(Q[0])
    m_chain()
    halo_next(Q[0], Q[1])
    proj_b(T, Q[1])
    attn(0, Q[0], O[0])

    def step(i, p, do_proj, do_attn):
        r0 = i * T if isinstance(i, int) else pl.multiple_of(i * T, T)
        if do_attn:
            if do_proj:
                halo_next(Q[p], Q[1 - p])
                proj_b(r0 + T, Q[1 - p])
            attn(None, Q[p], O[p])
        out_block(i - 1, r0 - T, O[1 - p])

    def body(m, _):
        step(2 * m + 1, 1, True, True)
        step(2 * m + 2, 0, True, True)
        return 0

    lax.fori_loop(0, (NB - 2) // 2, body, 0)
    step(NB - 1, 1, False, True)
    step(NB, 0, False, False)
    for i in range(NB):
        rows = pl.ds(i * T, T)
        pltpu.make_async_copy(ostage.at[rows, :], out_h.at[rows, :], osem.at[i]).wait()


@jax.jit
def pallas_concat_heads__linear_attn_block__sliding_local_dilated__prompt_kernel(
        A_x, A_wqkv, A_wo, B_x, B_wqkv, B_wo):
    xa = jnp.transpose(A_x, (0, 2, 1)).reshape(D, S)
    xb = jnp.transpose(B_x, (0, 2, 1)).reshape(D, S)
    hbm = pl.BlockSpec(memory_space=pl.ANY)
    out = pl.pallas_call(
        _kernel,
        out_shape=jax.ShapeDtypeStruct((S, 2 * D), BF16),
        in_specs=[hbm] * 6,
        out_specs=hbm,
        scratch_shapes=[
            pltpu.VMEM((D, S), BF16),
            pltpu.VMEM((D, S), BF16),
            pltpu.VMEM((D, 3 * D), BF16),
            pltpu.VMEM((D, 3 * D), BF16),
            pltpu.VMEM((D, D), BF16),
            pltpu.VMEM((D, D), BF16),
            pltpu.VMEM((5, 576, 128), U32),
            pltpu.VMEM((5, 864, 128), U32),
            pltpu.VMEM((5, 288, 128), U32),
            pltpu.VMEM((5, D // 2, 128), U32),
            pltpu.VMEM((5, D // 2, 128), U32),
            pltpu.VMEM((5, 896, 128), U32),
            pltpu.VMEM((5, DP // 2, 128), U32),
            pltpu.VMEM((5, D // 2, 128), U32),
            pltpu.VMEM((D, DP), F32),
            pltpu.VMEM((D, 128), F32),
            pltpu.VMEM((15, HALO + T, 128), F32),
            pltpu.VMEM((15, HALO + T, 128), F32),
            pltpu.VMEM((5, T // 2, 128), U32),
            pltpu.VMEM((5, T // 2, 128), U32),
            pltpu.VMEM((S, 2 * D), BF16),
            pltpu.SemaphoreType.DMA((9,)),
            pltpu.SemaphoreType.DMA((NB,)),
        ],
        compiler_params=pltpu.CompilerParams(vmem_limit_bytes=110 * 1024 * 1024),
    )(xa, A_wqkv, A_wo, xb, B_wqkv, B_wo)
    return out.reshape(1, S, 2 * D)
```

```python
import jax
import jax.numpy as jnp
import numpy as np
from jax import lax
import jax.experimental.pallas as pl
import jax.experimental.pallas.tpu as pltpu

S = 2048
D = 576
H = 32
DH = 18
DP = 640
WIN = 8
DIL = 2
HALO = 16
T1 = 512
SUB = 16
BLOCKS = (512, 512, 512, 256, 256)
XA0 = 512
XA1 = 1024
GH = 7
TMAX = max(BLOCKS)
F32 = jnp.float32
BF16 = jnp.bfloat16
U32 = jnp.uint32
NN = (((1,), (0,)), ((), ()))
NT = (((1,), (1,)), ((), ()))
QT = (0, 1, 2, 3, 8)
KT = (4, 5, 6, 7, 9)
VT = (10, 11, 12, 13, 14)


def _phi(t):
    return jnp.where(t > 0, t + 1.0, jnp.exp(t)) + 1e-6


def _dot(a, b, dims=NN):
    return lax.dot_general(a, b, dims, preferred_element_type=F32)


def _recip(d):
    r = pl.reciprocal(d, approx=True)
    return r * (2.0 - d * r)


def _ldw(ref, r0=None, r1=None):
    sl = slice(None) if r0 is None else slice(r0 // 2, r1 // 2)
    return pltpu.bitcast(jnp.concatenate([ref[j, sl, :] for j in range(5)], axis=1), BF16)


def _stw(ref, r0, val):
    u = pltpu.bitcast(val, U32)
    for j in range(5):
        ref[j, r0 // 2:r0 // 2 + u.shape[0], :] = u[:, 128 * j:128 * j + 128]


def _pad_lanes(v):
    return jnp.concatenate([v, jnp.zeros((v.shape[0], DP - v.shape[1]), v.dtype)], axis=1)


def _pad_rows(v, fill=0.0):
    return jnp.concatenate([v, jnp.full((DP - v.shape[0], v.shape[1]), fill, v.dtype)], axis=0)


def _kernel(xa_h, wa_h, woa_h, xb_h, wb_h, wob_h, out_h,
            xa_s, xb_s, wa_s, wb_s, woa_s, wob_s,
            ua, ub, uo, wk, wq, wb, wob, mt, ms, zs, zb, q0, q1, ostage,
            isem, osem):
    def cp(src, dst, k):
        return pltpu.make_async_copy(src, dst, isem.at[k])

    c_wak = cp(wa_h.at[:, 512:1152], wa_s.at[:, 512:1152], 0)
    c_xa0 = cp(xa_h.at[:, 0:XA0], xa_s.at[:, 0:XA0], 1)
    c_xa1 = cp(xa_h.at[:, XA0:XA1], xa_s.at[:, XA0:XA1], 2)
    c_xa2 = cp(xa_h.at[:, XA1:S], xa_s.at[:, XA1:S], 3)
    c_wb = cp(wb_h, wb_s, 4)
    c_xb0 = cp(xb_h.at[:, 0:512], xb_s.at[:, 0:512], 5)
    c_waq = cp(wa_h.at[:, 0:512], wa_s.at[:, 0:512], 6)
    c_wob = cp(wob_h, wob_s, 7)
    c_wav = cp(wa_h.at[:, 1152:1728], wa_s.at[:, 1152:1728], 8)
    c_woa = cp(woa_h, woa_s, 9)
    c_xb1 = cp(xb_h.at[:, 512:S], xb_s.at[:, 512:S], 10)
    for c in (c_wak, c_xa0, c_xa1, c_xa2, c_wb, c_xb0, c_waq, c_wob, c_wav, c_woa, c_xb1):
        c.start()

    def transposed_chunk(w_s, j):
        n = 128 if j < 13 else 64
        return _pad_lanes(w_s[:, 128 * j:128 * j + n].T)

    def transpose_chunks(w_s, u_s, chunks):
        for j in chunks:
            _stw(u_s, 128 * j, transposed_chunk(w_s, j))

    def perm_rows(u_s, base, dst, dst_row):
        for dp in range(DH // 2):
            for kt in range(5):
                a = u_s[kt, pl.ds(base + dp, 16, stride=DH), :]
                b = u_s[kt, pl.ds(base + dp + DH // 2, 16, stride=DH), :]
                r0 = dst_row(2 * dp) // 2
                r1 = dst_row(2 * dp + 1) // 2
                dst[kt, r0:r0 + 16, :] = (a & jnp.uint32(0xFFFF)) | (b << 16)
                dst[kt, r1:r1 + 16, :] = (a >> 16) | (b & jnp.uint32(0xFFFF0000))

    def brow(p):
        def f(d):
            if d < 16:
                return (0, 512, 1152)[p] + H * d
            return (1024, 1088, 1664)[p] + H * (d - 16)
        return f

    c_wak.wait()
    ct = transposed_chunk(wa_s, 4)
    _stw(ua, 512, ct[0:64])
    _stw(wk, 0, ct[64:128])
    for j in range(5, 9):
        _stw(wk, 128 * j - D, transposed_chunk(wa_s, j))

    n1 = S // T1
    pre = {i: [] for i in range(n1 + 1)}
    mid = {i: [] for i in range(n1 + 1)}
    pre[0] += [c_xa0.wait]
    pre[XA0 // T1] += [c_xa1.wait]
    b2 = XA1 // T1

    def wb_pad():
        for kt in range(5):
            wb[kt, 864:896, :] = jnp.zeros((32, 128), U32)

    pre[b2] += [c_xa2.wait, c_wb.wait]
    mid[b2] += [lambda: transpose_chunks(wb_s, ub, range(0, 5))]
    pre[b2 + 1] += [lambda: transpose_chunks(wb_s, ub, range(5, 10))]
    mid[b2 + 1] += [lambda: transpose_chunks(wb_s, ub, range(10, 14)), wb_pad]
    mid[b2 + 1] += [lambda: perm_rows(ub, 0, wb, brow(0)), lambda: perm_rows(ub, 288, wb, brow(1)),
                    lambda: perm_rows(ub, 576, wb, brow(2))]

    g_acc = None
    for i in range(n1):
        for t in pre[i]:
            t()
        xt = xa_s[:, i * T1:(i + 1) * T1]
        pkt = _phi(_dot(_ldw(wk), _pad_rows(xt))).astype(BF16)
        for t in mid[i]:
            t()
        g = _dot(pkt, _pad_rows(xt, 1.0), NT)
        g_acc = g if i == 0 else g_acc + g

    def m_chain():
        for c in range(-(-H // GH)):
            f0 = GH * DH * c
            n = min(128, D - f0)
            cc = _dot(g_acc[f0:f0 + n, 0:D].astype(BF16), wa_s[:, 1152 + f0:1152 + f0 + n])
            row = lax.broadcasted_iota(jnp.int32, (n, n), 0)
            col = lax.broadcasted_iota(jnp.int32, (n, n), 1)
            keep = None
            for a in range(GH):
                lo = a * DH
                blk = (row >= lo) & (row < lo + DH) & (col >= lo) & (col < lo + DH)
                keep = blk if keep is None else keep | blk
            cc = jnp.where(keep, cc, 0.0).astype(BF16)
            mc = _dot(cc, woa_s[f0:f0 + n, :])
            nr = min(GH * DH, n)
            mc = _pad_lanes(mc[0:nr])
            for kt in range(5):
                ms[kt, f0:f0 + nr, :] = mc[:, 128 * kt:128 * kt + 128]
        gt = g_acc[:, 512:DP]
        lane = lax.broadcasted_iota(jnp.int32, (D, 128), 1)
        zs[...] = jnp.where(lane < 64, pltpu.roll(gt, 64, 1), gt)
        rows = []
        for d in range(DH):
            sl = pl.ds(d, H, stride=DH)
            zb[H * d:H * d + H, :] = zs[sl, :]
            rows.append(jnp.concatenate([ms[kt, sl, :] for kt in range(5)], axis=1)[:, 0:D])
        mfull = jnp.concatenate(rows, axis=0)
        _stw(mt, 0, _pad_lanes(mfull.astype(BF16).T))

    def prep_wob():
        w = jnp.concatenate([jnp.zeros((D, 64), BF16), wob_s[...]], axis=1)
        _stw(uo, 0, w)
        perm_rows(uo, 0, wob, lambda d: H * d)
        for kt in range(5):
            wob[kt, D // 2:DP // 2, :] = jnp.zeros((32, 128), U32)

    cscale = np.float32(DH ** -0.5 * np.log2(np.e))

    def proj_b(r0, t, qkv):
        x = _pad_rows(xb_s[:, r0:r0 + t]).T
        body = pl.ds(HALO, t)
        r = _dot(x, _ldw(wb), NT)
        for j in range(4):
            qkv[j, body, :] = r[:, 128 * j:128 * j + 128] * cscale
        for j in range(4, 8):
            qkv[j, body, :] = r[:, 128 * j:128 * j + 128]
        tail = r[:, 1024:1152]
        lane = lax.broadcasted_iota(jnp.int32, (t, 128), 1)
        qkv[8, body, :] = jnp.where(lane < 64, tail * cscale, 0.0)
        qkv[9, body, :] = pltpu.roll(tail, 64, 1)
        for j in range(9, 14):
            qkv[j + 1, body, :] = r[:, 128 * j:128 * j + 128]

    def halo_first(qkv):
        for j in KT + VT:
            qkv[j, 0:HALO, :] = jnp.broadcast_to(qkv[j, HALO:HALO + 1, :], (HALO, 128))

    def halo_next(src, t, dst):
        for j in KT + VT:
            dst[j, 0:HALO, :] = src[j, t:t + HALO, :]

    def attn(first, t, qkv):
        outs = []
        for s in range(t // SUB):
            base = s * SUB
            q = [qkv[j, pl.ds(HALO + base, SUB), :] for j in QT]
            logits = []
            for w in range(WIN):
                sh = HALO - DIL * w
                acc = q[0] * qkv[KT[0], pl.ds(base + sh, SUB), :]
                for j in range(1, 5):
                    acc = acc + q[j] * qkv[KT[j], pl.ds(base + sh, SUB), :]
                acc = acc + pltpu.roll(acc, 64, 1)
                acc = acc + pltpu.roll(acc, 32, 1)
                if first and s * SUB < DIL * w:
                    pos = base + lax.broadcasted_iota(jnp.int32, (SUB, 128), 0)
                    acc = jnp.where(pos >= DIL * w, acc, -1e9 * float(np.log2(np.e)))
                logits.append(acc)
            m = logits[0]
            for w in range(1, WIN):
                m = jnp.maximum(m, logits[w])
            es = [jnp.exp2(l - m) for l in logits]
            den = es[0]
            for w in range(1, WIN):
                den = den + es[w]
            inv = _recip(den)
            row = []
            for j in range(5):
                acc = es[0] * qkv[VT[j], pl.ds(base + HALO, SUB), :]
                for w in range(1, WIN):
                    acc = acc + es[w] * qkv[VT[j], pl.ds(base + HALO - DIL * w, SUB), :]
                row.append(acc * inv)
            outs.append(jnp.concatenate(row, axis=1))
        return jnp.concatenate(outs, axis=0).astype(BF16)

    def a_q(r0, t):
        pq = _phi(_dot(_ldw(wq), _pad_rows(xa_s[:, r0:r0 + t])))
        pz = pq * jnp.concatenate([zb[...]] * (t // 128), axis=1)
        den = pz[0:H]
        for d in range(1, DH):
            den = den + pz[H * d:H * d + H]
        inv = _recip(den + 1e-6)
        return jnp.concatenate([pq[H * d:H * d + H] * inv for d in range(DH)], axis=0).astype(BF16)

    def out_copy(i):
        rows = pl.ds(starts[i], BLOCKS[i])
        return pltpu.make_async_copy(ostage.at[rows, :], out_h.at[rows, :], osem.at[i])

    def out_block(i, pqs, ob):
        rows = pl.ds(starts[i], BLOCKS[i])
        rb = _dot(ob, _ldw(wob)).astype(BF16)
        ostage[rows, D:640] = rb[:, 64:128]
        ostage[rows, 640:2 * D] = rb[:, 128:DP]
        oat = _dot(_ldw(mt), _pad_rows(pqs))
        ostage[rows, 0:D] = oat.T.astype(BF16)
        out_copy(i).start()

    nb = len(BLOCKS)
    starts = [sum(BLOCKS[:i]) for i in range(nb)]
    Q = (q0, q1)
    for c in (c_xb0, c_waq, c_wob, c_wav, c_woa, c_xb1):
        c.wait()
    proj_b(0, BLOCKS[0], Q[0])
    transpose_chunks(wa_s, ua, range(0, 4))
    perm_rows(ua, 0, wq, lambda d: H * d)
    halo_first(Q[0])
    m_chain()
    prep_wob()
    carry = None
    for i in range(nb):
        p = i % 2
        if carry is not None:
            out_block(i - 1, *carry)
        if i + 1 < nb:
            halo_next(Q[p], BLOCKS[i], Q[1 - p])
            proj_b(starts[i + 1], BLOCKS[i + 1], Q[1 - p])
        carry = (a_q(starts[i], BLOCKS[i]), attn(i == 0, BLOCKS[i], Q[p]))
    out_block(nb - 1, *carry)
    for i in range(nb):
        out_copy(i).wait()


@jax.jit
def pallas_concat_heads__linear_attn_block__sliding_local_dilated__prompt_kernel(
        A_x, A_wqkv, A_wo, B_x, B_wqkv, B_wo):
    xa = jnp.transpose(A_x, (0, 2, 1)).reshape(D, S)
    xb = jnp.transpose(B_x, (0, 2, 1)).reshape(D, S)
    hbm = pl.BlockSpec(memory_space=pl.ANY)
    out = pl.pallas_call(
        _kernel,
        out_shape=jax.ShapeDtypeStruct((S, 2 * D), BF16),
        in_specs=[hbm] * 6,
        out_specs=hbm,
        scratch_shapes=[
            pltpu.VMEM((D, S), BF16),
            pltpu.VMEM((D, S), BF16),
            pltpu.VMEM((D, 3 * D), BF16),
            pltpu.VMEM((D, 3 * D), BF16),
            pltpu.VMEM((D, D), BF16),
            pltpu.VMEM((D, D), BF16),
            pltpu.VMEM((5, D // 2, 128), U32),
            pltpu.VMEM((5, 864, 128), U32),
            pltpu.VMEM((5, D // 2, 128), U32),
            pltpu.VMEM((5, D // 2, 128), U32),
            pltpu.VMEM((5, D // 2, 128), U32),
            pltpu.VMEM((5, 896, 128), U32),
            pltpu.VMEM((5, DP // 2, 128), U32),
            pltpu.VMEM((5, D // 2, 128), U32),
            pltpu.VMEM((5, D, 128), F32),
            pltpu.VMEM((D, 128), F32),
            pltpu.VMEM((D, 128), F32),
            pltpu.VMEM((15, HALO + TMAX, 128), F32),
            pltpu.VMEM((15, HALO + TMAX, 128), F32),
            pltpu.VMEM((S, 2 * D), BF16),
            pltpu.SemaphoreType.DMA((11,)),
            pltpu.SemaphoreType.DMA((len(BLOCKS),)),
        ],
        compiler_params=pltpu.CompilerParams(
            vmem_limit_bytes=110 * 1024 * 1024,
            flags={"XLA_TPU_EVENLY_DISTRIBUTE_CRITICAL_NODES": True}),
    )(xa, A_wqkv, A_wo, xb, B_wqkv, B_wo)
    return out.reshape(1, S, 2 * D)
```

```python
import jax
import jax.numpy as jnp
import numpy as np
from jax import lax
import jax.experimental.pallas as pl
import jax.experimental.pallas.tpu as pltpu

S = 2048
D = 576
H = 32
DH = 18
DP = 640
WIN = 8
DIL = 2
HALO = 16
SUB = 16
BLOCKS = (512, 512, 512, 512)
LAST = (256, 128, 128)
P1B = (512, 512, 512, 512)
XA0 = 512
XA1 = 1024
GH = 7
TMAX = max(BLOCKS)
F32 = jnp.float32
BF16 = jnp.bfloat16
U32 = jnp.uint32
NN = (((1,), (0,)), ((), ()))
NT = (((1,), (1,)), ((), ()))
QT = (0, 1, 2, 3, 8)
KT = (4, 5, 6, 7, 9)
VT = (10, 11, 12, 13, 14)


def _phi(t):
    return jnp.where(t > 0, t + 1.0, jnp.exp(t)) + 1e-6


def _dot(a, b, dims=NN):
    return lax.dot_general(a, b, dims, preferred_element_type=F32)


def _recip(d):
    r = pl.reciprocal(d, approx=True)
    return r * (2.0 - d * r)


def _ldw(ref, r0=None, r1=None):
    sl = slice(None) if r0 is None else slice(r0 // 2, r1 // 2)
    return pltpu.bitcast(jnp.concatenate([ref[j, sl, :] for j in range(5)], axis=1), BF16)


def _stw(ref, r0, val):
    u = pltpu.bitcast(val, U32)
    for j in range(5):
        ref[j, r0 // 2:r0 // 2 + u.shape[0], :] = u[:, 128 * j:128 * j + 128]


def _pad_lanes(v):
    return jnp.concatenate([v, jnp.zeros((v.shape[0], DP - v.shape[1]), v.dtype)], axis=1)


def _pad_rows(v, fill=0.0):
    return jnp.concatenate([v, jnp.full((DP - v.shape[0], v.shape[1]), fill, v.dtype)], axis=0)


def _kernel(xa_h, wa_h, woa_h, xb_h, wb_h, wob_h, out_h,
            xa_s, xb_s, wa_s, wb_s, woa_s, wob_s,
            ua, ub, uo, wk, wq, wb, wob, mt, ms, zs, zb, q0, q1, ostage,
            isem, osem):
    def cp(src, dst, k):
        return pltpu.make_async_copy(src, dst, isem.at[k])

    c_wak = cp(wa_h.at[:, 512:1152], wa_s.at[:, 512:1152], 0)
    c_xa0 = cp(xa_h.at[:, 0:XA0], xa_s.at[:, 0:XA0], 1)
    c_xa1 = cp(xa_h.at[:, XA0:XA1], xa_s.at[:, XA0:XA1], 2)
    c_xa2 = cp(xa_h.at[:, XA1:S], xa_s.at[:, XA1:S], 3)
    c_wb = cp(wb_h, wb_s, 4)
    c_xb0 = cp(xb_h.at[:, 0:512], xb_s.at[:, 0:512], 5)
    c_waq = cp(wa_h.at[:, 0:512], wa_s.at[:, 0:512], 6)
    c_wob = cp(wob_h, wob_s, 7)
    c_wav = cp(wa_h.at[:, 1152:1728], wa_s.at[:, 1152:1728], 8)
    c_woa = cp(woa_h, woa_s, 9)
    c_xb1 = cp(xb_h.at[:, 512:S], xb_s.at[:, 512:S], 10)
    for c in (c_wak, c_xa0, c_xa1, c_xa2, c_wb, c_xb0, c_waq, c_wob, c_wav, c_woa, c_xb1):
        c.start()

    def transposed_chunk(w_s, j):
        n = 128 if j < 13 else 64
        return _pad_lanes(w_s[:, 128 * j:128 * j + n].T)

    def transpose_chunks(w_s, u_s, chunks):
        for j in chunks:
            _stw(u_s, 128 * j, transposed_chunk(w_s, j))

    def perm_rows(u_s, base, dst, dst_row):
        for dp in range(DH // 2):
            for kt in range(5):
                a = u_s[kt, pl.ds(base + dp, 16, stride=DH), :]
                b = u_s[kt, pl.ds(base + dp + DH // 2, 16, stride=DH), :]
                r0 = dst_row(2 * dp) // 2
                r1 = dst_row(2 * dp + 1) // 2
                dst[kt, r0:r0 + 16, :] = (a & jnp.uint32(0xFFFF)) | (b << 16)
                dst[kt, r1:r1 + 16, :] = (a >> 16) | (b & jnp.uint32(0xFFFF0000))

    def brow(p):
        def f(d):
            if d < 16:
                return (0, 512, 1152)[p] + H * d
            return (1024, 1088, 1664)[p] + H * (d - 16)
        return f

    c_wak.wait()
    ct = transposed_chunk(wa_s, 4)
    _stw(ua, 512, ct[0:64])
    _stw(wk, 0, ct[64:128])
    for j in range(5, 9):
        _stw(wk, 128 * j - D, transposed_chunk(wa_s, j))

    n1 = len(P1B)
    st1 = [sum(P1B[:i]) for i in range(n1)]
    pre = {i: [] for i in range(n1 + 1)}
    mid = {i: [] for i in range(n1 + 1)}
    pre[0] += [c_xa0.wait]
    pre[st1.index(XA0)] += [c_xa1.wait]
    b2 = st1.index(XA1)

    def wb_pad():
        for kt in range(5):
            wb[kt, 864:896, :] = jnp.zeros((32, 128), U32)

    pre[b2] += [c_xa2.wait, c_wb.wait]
    mid[b2] += [lambda: transpose_chunks(wb_s, ub, range(0, 5))]
    pre[b2 + 1] += [lambda: transpose_chunks(wb_s, ub, range(5, 10))]
    mid[b2 + 1] += [lambda: transpose_chunks(wb_s, ub, range(10, 14)), wb_pad]
    mid[b2 + 1] += [lambda: perm_rows(ub, 0, wb, brow(0)), lambda: perm_rows(ub, 288, wb, brow(1)),
                    lambda: perm_rows(ub, 576, wb, brow(2))]

    g_acc = None
    for i in range(n1):
        for t in pre[i]:
            t()
        xt = xa_s[:, st1[i]:st1[i] + P1B[i]]
        pkt = _phi(_dot(_ldw(wk), _pad_rows(xt))).astype(BF16)
        for t in mid[i]:
            t()
        g = _dot(pkt, _pad_rows(xt, 1.0), NT)
        g_acc = g if i == 0 else g_acc + g

    def m_chain():
        for c in range(-(-H // GH)):
            f0 = GH * DH * c
            n = min(128, D - f0)
            cc = _dot(g_acc[f0:f0 + n, 0:D].astype(BF16), wa_s[:, 1152 + f0:1152 + f0 + n])
            row = lax.broadcasted_iota(jnp.int32, (n, n), 0)
            col = lax.broadcasted_iota(jnp.int32, (n, n), 1)
            keep = None
            for a in range(GH):
                lo = a * DH
                blk = (row >= lo) & (row < lo + DH) & (col >= lo) & (col < lo + DH)
                keep = blk if keep is None else keep | blk
            cc = jnp.where(keep, cc, 0.0).astype(BF16)
            mc = _dot(cc, woa_s[f0:f0 + n, :])
            nr = min(GH * DH, n)
            mc = _pad_lanes(mc[0:nr])
            for kt in range(5):
                ms[kt, f0:f0 + nr, :] = mc[:, 128 * kt:128 * kt + 128]
        gt = g_acc[:, 512:DP]
        lane = lax.broadcasted_iota(jnp.int32, (D, 128), 1)
        zs[...] = jnp.where(lane < 64, pltpu.roll(gt, 64, 1), gt)
        rows = []
        for d in range(DH):
            sl = pl.ds(d, H, stride=DH)
            zb[H * d:H * d + H, :] = zs[sl, :]
            rows.append(jnp.concatenate([ms[kt, sl, :] for kt in range(5)], axis=1)[:, 0:D])
        mfull = jnp.concatenate(rows, axis=0)
        _stw(mt, 0, _pad_lanes(mfull.astype(BF16).T))

    def prep_wob():
        w = jnp.concatenate([jnp.zeros((D, 64), BF16), wob_s[...]], axis=1)
        _stw(uo, 0, w)
        perm_rows(uo, 0, wob, lambda d: H * d)
        for kt in range(5):
            wob[kt, D // 2:DP // 2, :] = jnp.zeros((32, 128), U32)

    cscale = np.float32(DH ** -0.5 * np.log2(np.e))

    def proj_b(r0, t, qkv):
        x = _pad_rows(xb_s[:, r0:r0 + t]).T
        body = pl.ds(HALO, t)
        r = _dot(x, _ldw(wb), NT)
        for j in range(4):
            qkv[j, body, :] = r[:, 128 * j:128 * j + 128] * cscale
        for j in range(4, 8):
            qkv[j, body, :] = r[:, 128 * j:128 * j + 128]
        tail = r[:, 1024:1152]
        lane = lax.broadcasted_iota(jnp.int32, (t, 128), 1)
        qkv[8, body, :] = jnp.where(lane < 64, tail * cscale, 0.0)
        qkv[9, body, :] = pltpu.roll(tail, 64, 1)
        for j in range(9, 14):
            qkv[j + 1, body, :] = r[:, 128 * j:128 * j + 128]

    def halo_first(qkv):
        for j in KT + VT:
            qkv[j, 0:HALO, :] = jnp.broadcast_to(qkv[j, HALO:HALO + 1, :], (HALO, 128))

    def halo_next(src, t, dst):
        for j in KT + VT:
            dst[j, 0:HALO, :] = src[j, t:t + HALO, :]

    def attn(first, t, qkv):
        outs = []
        for s in range(t // SUB):
            base = s * SUB
            q = [qkv[j, pl.ds(HALO + base, SUB), :] for j in QT]
            logits = []
            for w in range(WIN):
                sh = HALO - DIL * w
                acc = q[0] * qkv[KT[0], pl.ds(base + sh, SUB), :]
                for j in range(1, 5):
                    acc = acc + q[j] * qkv[KT[j], pl.ds(base + sh, SUB), :]
                acc = acc + pltpu.roll(acc, 64, 1)
                acc = acc + pltpu.roll(acc, 32, 1)
                if first and s * SUB < DIL * w:
                    pos = base + lax.broadcasted_iota(jnp.int32, (SUB, 128), 0)
                    acc = jnp.where(pos >= DIL * w, acc, -1e9 * float(np.log2(np.e)))
                logits.append(acc)
            m = logits[0]
            for w in range(1, WIN):
                m = jnp.maximum(m, logits[w])
            es = [jnp.exp2(l - m) for l in logits]
            den = es[0]
            for w in range(1, WIN):
                den = den + es[w]
            inv = _recip(den)
            row = []
            for j in range(5):
                acc = es[0] * qkv[VT[j], pl.ds(base + HALO, SUB), :]
                for w in range(1, WIN):
                    acc = acc + es[w] * qkv[VT[j], pl.ds(base + HALO - DIL * w, SUB), :]
                row.append(acc * inv)
            outs.append(jnp.concatenate(row, axis=1))
        return jnp.concatenate(outs, axis=0).astype(BF16)

    def a_q(r0, t):
        pq = _phi(_dot(_ldw(wq), _pad_rows(xa_s[:, r0:r0 + t])))
        pz = pq * jnp.concatenate([zb[...]] * (t // 128), axis=1)
        den = pz[0:H]
        for d in range(1, DH):
            den = den + pz[H * d:H * d + H]
        inv = _recip(den + 1e-6)
        return jnp.concatenate([pq[H * d:H * d + H] * inv for d in range(DH)], axis=0).astype(BF16)

    def out_copy(u, r0, t):
        rows = pl.ds(r0, t)
        return pltpu.make_async_copy(ostage.at[rows, :], out_h.at[rows, :], osem.at[u])

    copies = []

    def out_block(i, pqs, ob):
        parts = LAST if i == len(BLOCKS) - 1 else (BLOCKS[i],)
        for n, t in enumerate(parts):
            o = sum(parts[:n])
            rows = pl.ds(starts[i] + o, t)
            rb = _dot(ob[o:o + t], _ldw(wob)).astype(BF16)
            ostage[rows, D:640] = rb[:, 64:128]
            ostage[rows, 640:2 * D] = rb[:, 128:DP]
            oat = _dot(_ldw(mt), _pad_rows(pqs[:, o:o + t]))
            ostage[rows, 0:D] = oat.T.astype(BF16)
            c = out_copy(len(copies), starts[i] + o, t)
            copies.append(c)
            c.start()

    nb = len(BLOCKS)
    starts = [sum(BLOCKS[:i]) for i in range(nb)]
    Q = (q0, q1)
    for c in (c_xb0, c_waq, c_wob, c_wav, c_woa, c_xb1):
        c.wait()
    proj_b(0, BLOCKS[0], Q[0])
    transpose_chunks(wa_s, ua, range(0, 4))
    perm_rows(ua, 0, wq, lambda d: H * d)
    halo_first(Q[0])
    m_chain()
    prep_wob()
    carry = None
    for i in range(nb):
        p = i % 2
        if carry is not None:
            out_block(i - 1, *carry)
        if i + 1 < nb:
            halo_next(Q[p], BLOCKS[i], Q[1 - p])
            proj_b(starts[i + 1], BLOCKS[i + 1], Q[1 - p])
        carry = (a_q(starts[i], BLOCKS[i]), attn(i == 0, BLOCKS[i], Q[p]))
    out_block(nb - 1, *carry)
    for c in copies:
        c.wait()


@jax.jit
def pallas_concat_heads__linear_attn_block__sliding_local_dilated__prompt_kernel(
        A_x, A_wqkv, A_wo, B_x, B_wqkv, B_wo):
    xa = jnp.transpose(A_x, (0, 2, 1)).reshape(D, S)
    xb = jnp.transpose(B_x, (0, 2, 1)).reshape(D, S)
    hbm = pl.BlockSpec(memory_space=pl.ANY)
    out = pl.pallas_call(
        _kernel,
        out_shape=jax.ShapeDtypeStruct((S, 2 * D), BF16),
        in_specs=[hbm] * 6,
        out_specs=hbm,
        scratch_shapes=[
            pltpu.VMEM((D, S), BF16),
            pltpu.VMEM((D, S), BF16),
            pltpu.VMEM((D, 3 * D), BF16),
            pltpu.VMEM((D, 3 * D), BF16),
            pltpu.VMEM((D, D), BF16),
            pltpu.VMEM((D, D), BF16),
            pltpu.VMEM((5, D // 2, 128), U32),
            pltpu.VMEM((5, 864, 128), U32),
            pltpu.VMEM((5, D // 2, 128), U32),
            pltpu.VMEM((5, D // 2, 128), U32),
            pltpu.VMEM((5, D // 2, 128), U32),
            pltpu.VMEM((5, 896, 128), U32),
            pltpu.VMEM((5, DP // 2, 128), U32),
            pltpu.VMEM((5, D // 2, 128), U32),
            pltpu.VMEM((5, D, 128), F32),
            pltpu.VMEM((D, 128), F32),
            pltpu.VMEM((D, 128), F32),
            pltpu.VMEM((15, HALO + TMAX, 128), F32),
            pltpu.VMEM((15, HALO + TMAX, 128), F32),
            pltpu.VMEM((S, 2 * D), BF16),
            pltpu.SemaphoreType.DMA((11,)),
            pltpu.SemaphoreType.DMA((len(BLOCKS) + len(LAST) - 1,)),
        ],
        compiler_params=pltpu.CompilerParams(
            vmem_limit_bytes=110 * 1024 * 1024,
            flags={"XLA_TPU_EVENLY_DISTRIBUTE_CRITICAL_NODES": True}),
    )(xa, A_wqkv, A_wo, xb, B_wqkv, B_wo)
    return out.reshape(1, S, 2 * D)
```

```python
import jax
import jax.numpy as jnp
import numpy as np
from jax import lax
import jax.experimental.pallas as pl
import jax.experimental.pallas.tpu as pltpu

S = 2048
D = 576
H = 32
DH = 18
DP = 640
WIN = 8
DIL = 2
HALO = 16
SUB = 16
BLOCKS = (512, 512, 512, 512)
LAST = (256, 128, 128)
P1B = (512, 512, 512, 512)
XA0 = 512
XA1 = 1024
GH = 7
TMAX = max(BLOCKS)
F32 = jnp.float32
BF16 = jnp.bfloat16
U32 = jnp.uint32
NN = (((1,), (0,)), ((), ()))
NT = (((1,), (1,)), ((), ()))
QT = (0, 1, 2, 3, 8)
KT = (4, 5, 6, 7, 9)
VT = (10, 11, 12, 13, 14)


def _phi(t):
    return jnp.where(t > 0, t + 1.0, jnp.exp(t)) + 1e-6


def _dot(a, b, dims=NN):
    return lax.dot_general(a, b, dims, preferred_element_type=F32)


def _recip(d):
    r = pl.reciprocal(d, approx=True)
    return r * (2.0 - d * r)


def _ldw(ref, r0=None, r1=None):
    sl = slice(None) if r0 is None else slice(r0 // 2, r1 // 2)
    return pltpu.bitcast(jnp.concatenate([ref[j, sl, :] for j in range(5)], axis=1), BF16)


def _stw(ref, r0, val):
    u = pltpu.bitcast(val, U32)
    for j in range(5):
        ref[j, r0 // 2:r0 // 2 + u.shape[0], :] = u[:, 128 * j:128 * j + 128]


def _pad_lanes(v):
    return jnp.concatenate([v, jnp.zeros((v.shape[0], DP - v.shape[1]), v.dtype)], axis=1)


def _pad_rows(v, fill=0.0):
    return jnp.concatenate([v, jnp.full((DP - v.shape[0], v.shape[1]), fill, v.dtype)], axis=0)


def _kernel(xa_h, wa_h, woa_h, xb_h, wb_h, wob_h, out_h,
            xa_s, xb_s, wa_s, wb_s, woa_s, wob_s,
            ua, ub, uo, wk, wq, wb, wob, mt, ms, zs, zb, q0, q1, ostage,
            isem, osem):
    def cp(src, dst, k):
        return pltpu.make_async_copy(src, dst, isem.at[k])

    c_wak = cp(wa_h.at[:, 512:1152], wa_s.at[:, 512:1152], 0)
    c_xa0 = cp(xa_h.at[:, 0:XA0], xa_s.at[:, 0:XA0], 1)
    c_xa1 = cp(xa_h.at[:, XA0:XA1], xa_s.at[:, XA0:XA1], 2)
    c_xa2 = cp(xa_h.at[:, XA1:S], xa_s.at[:, XA1:S], 3)
    c_wb = cp(wb_h, wb_s, 4)
    c_xb0 = cp(xb_h.at[:, 0:512], xb_s.at[:, 0:512], 5)
    c_waq = cp(wa_h.at[:, 0:512], wa_s.at[:, 0:512], 6)
    c_wob = cp(wob_h, wob_s, 7)
    c_wav = cp(wa_h.at[:, 1152:1728], wa_s.at[:, 1152:1728], 8)
    c_woa = cp(woa_h, woa_s, 9)
    c_xb1 = cp(xb_h.at[:, 512:S], xb_s.at[:, 512:S], 10)
    for c in (c_wak, c_xa0, c_xa1, c_xa2, c_wb, c_xb0, c_waq, c_wob, c_wav, c_woa, c_xb1):
        c.start()

    def transposed_chunk(w_s, j):
        n = 128 if j < 13 else 64
        return _pad_lanes(w_s[:, 128 * j:128 * j + n].T)

    def transpose_chunks(w_s, u_s, chunks):
        for j in chunks:
            _stw(u_s, 128 * j, transposed_chunk(w_s, j))

    def perm_rows(u_s, base, dst, dst_row):
        for dp in range(DH // 2):
            for kt in range(5):
                a = u_s[kt, pl.ds(base + dp, 16, stride=DH), :]
                b = u_s[kt, pl.ds(base + dp + DH // 2, 16, stride=DH), :]
                r0 = dst_row(2 * dp) // 2
                r1 = dst_row(2 * dp + 1) // 2
                dst[kt, r0:r0 + 16, :] = (a & jnp.uint32(0xFFFF)) | (b << 16)
                dst[kt, r1:r1 + 16, :] = (a >> 16) | (b & jnp.uint32(0xFFFF0000))

    def brow(p):
        def f(d):
            if d < 16:
                return (0, 512, 1152)[p] + H * d
            return (1024, 1088, 1664)[p] + H * (d - 16)
        return f

    c_wak.wait()
    ct = transposed_chunk(wa_s, 4)
    _stw(ua, 512, ct[0:64])
    _stw(wk, 0, ct[64:128])
    for j in range(5, 9):
        _stw(wk, 128 * j - D, transposed_chunk(wa_s, j))

    n1 = len(P1B)
    st1 = [sum(P1B[:i]) for i in range(n1)]
    pre = {i: [] for i in range(n1 + 1)}
    mid = {i: [] for i in range(n1 + 1)}
    pre[0] += [c_xa0.wait]
    pre[st1.index(XA0)] += [c_xa1.wait]
    b2 = st1.index(XA1)

    def wb_pad():
        for kt in range(5):
            wb[kt, 864:896, :] = jnp.zeros((32, 128), U32)

    pre[b2] += [c_xa2.wait, c_wb.wait]
    mid[b2] += [lambda: transpose_chunks(wb_s, ub, range(0, 5))]
    pre[b2 + 1] += [lambda: transpose_chunks(wb_s, ub, range(5, 10))]
    mid[b2 + 1] += [lambda: transpose_chunks(wb_s, ub, range(10, 14)), wb_pad]
    mid[b2 + 1] += [lambda: perm_rows(ub, 0, wb, brow(0)), lambda: perm_rows(ub, 288, wb, brow(1)),
                    lambda: perm_rows(ub, 576, wb, brow(2))]

    g_acc = None
    for i in range(n1):
        for t in pre[i]:
            t()
        xt = xa_s[:, st1[i]:st1[i] + P1B[i]]
        pkt = _phi(_dot(_ldw(wk), _pad_rows(xt))).astype(BF16)
        for t in mid[i]:
            t()
        g = _dot(pkt, _pad_rows(xt, 1.0), NT)
        g_acc = g if i == 0 else g_acc + g

    def m_chain():
        for c in range(-(-H // GH)):
            f0 = GH * DH * c
            n = min(128, D - f0)
            cc = _dot(g_acc[f0:f0 + n, 0:D].astype(BF16), wa_s[:, 1152 + f0:1152 + f0 + n])
            row = lax.broadcasted_iota(jnp.int32, (n, n), 0)
            col = lax.broadcasted_iota(jnp.int32, (n, n), 1)
            keep = None
            for a in range(GH):
                lo = a * DH
                blk = (row >= lo) & (row < lo + DH) & (col >= lo) & (col < lo + DH)
                keep = blk if keep is None else keep | blk
            cc = jnp.where(keep, cc, 0.0).astype(BF16)
            mc = _dot(cc, woa_s[f0:f0 + n, :])
            nr = min(GH * DH, n)
            mc = _pad_lanes(mc[0:nr])
            for kt in range(5):
                ms[kt, f0:f0 + nr, :] = mc[:, 128 * kt:128 * kt + 128]
        gt = g_acc[:, 512:DP]
        lane = lax.broadcasted_iota(jnp.int32, (D, 128), 1)
        zs[0:D, :] = jnp.where(lane < 64, pltpu.roll(gt, 64, 1), gt)
        rows = []
        for d in range(DH):
            sl = pl.ds(d, H, stride=DH)
            zb[H * d:H * d + H, :] = zs[sl, :]
            rows.append(jnp.concatenate([ms[kt, sl, :] for kt in range(5)], axis=1)[:, 0:D])
        mfull = jnp.concatenate(rows, axis=0)
        _stw(mt, 0, _pad_lanes(mfull.astype(BF16).T))

    def prep_wob():
        w = jnp.concatenate([jnp.zeros((D, 64), BF16), wob_s[...]], axis=1)
        _stw(uo, 0, w)
        perm_rows(uo, 0, wob, lambda d: H * d)
        for kt in range(5):
            wob[kt, D // 2:DP // 2, :] = jnp.zeros((32, 128), U32)

    cscale = np.float32(DH ** -0.5 * np.log2(np.e))

    def proj_b(r0, t, qkv):
        x = _pad_rows(xb_s[:, r0:r0 + t]).T
        body = pl.ds(HALO, t)
        r = _dot(x, _ldw(wb), NT)
        for j in range(4):
            qkv[j, body, :] = r[:, 128 * j:128 * j + 128] * cscale
        for j in range(4, 8):
            qkv[j, body, :] = r[:, 128 * j:128 * j + 128]
        tail = r[:, 1024:1152]
        lane = lax.broadcasted_iota(jnp.int32, (t, 128), 1)
        qkv[8, body, :] = jnp.where(lane < 64, tail * cscale, 0.0)
        qkv[9, body, :] = pltpu.roll(tail, 64, 1)
        for j in range(9, 14):
            qkv[j + 1, body, :] = r[:, 128 * j:128 * j + 128]

    def halo_first(qkv):
        for j in KT + VT:
            qkv[j, 0:HALO, :] = jnp.broadcast_to(qkv[j, HALO:HALO + 1, :], (HALO, 128))

    def halo_next(src, t, dst):
        for j in KT + VT:
            dst[j, 0:HALO, :] = src[j, t:t + HALO, :]

    def attn(first, t, qkv):
        outs = []
        for s in range(t // SUB):
            base = s * SUB
            q = [qkv[j, pl.ds(HALO + base, SUB), :] for j in QT]
            logits = []
            for w in range(WIN):
                sh = HALO - DIL * w
                acc = q[0] * qkv[KT[0], pl.ds(base + sh, SUB), :]
                for j in range(1, 5):
                    acc = acc + q[j] * qkv[KT[j], pl.ds(base + sh, SUB), :]
                acc = acc + pltpu.roll(acc, 64, 1)
                acc = acc + pltpu.roll(acc, 32, 1)
                if first and s * SUB < DIL * w:
                    pos = base + lax.broadcasted_iota(jnp.int32, (SUB, 128), 0)
                    acc = jnp.where(pos >= DIL * w, acc, -1e9 * float(np.log2(np.e)))
                logits.append(acc)
            m = logits[0]
            for w in range(1, WIN):
                m = jnp.maximum(m, logits[w])
            es = [jnp.exp2(l - m) for l in logits]
            den = es[0]
            for w in range(1, WIN):
                den = den + es[w]
            inv = _recip(den)
            row = []
            for j in range(5):
                acc = es[0] * qkv[VT[j], pl.ds(base + HALO, SUB), :]
                for w in range(1, WIN):
                    acc = acc + es[w] * qkv[VT[j], pl.ds(base + HALO - DIL * w, SUB), :]
                row.append(acc * inv)
            outs.append(jnp.concatenate(row, axis=1))
        return jnp.concatenate(outs, axis=0).astype(BF16)

    def a_q(r0, t):
        pq = _phi(_dot(_ldw(wq), _pad_rows(xa_s[:, r0:r0 + t])))
        pz = pq * jnp.concatenate([zb[...]] * (t // 128), axis=1)
        den = pz[0:H]
        for d in range(1, DH):
            den = den + pz[H * d:H * d + H]
        inv = _recip(den + 1e-6)
        return jnp.concatenate([pq[H * d:H * d + H] * inv for d in range(DH)], axis=0).astype(BF16)

    def out_copy(u, r0, t):
        rows = pl.ds(r0, t)
        return pltpu.make_async_copy(ostage.at[rows, :], out_h.at[rows, :], osem.at[u])

    copies = []

    def out_block(i, pqs, ob):
        parts = LAST if i == len(BLOCKS) - 1 else (BLOCKS[i],)
        for n, t in enumerate(parts):
            o = sum(parts[:n])
            rows = pl.ds(starts[i] + o, t)
            rb = _dot(ob[o:o + t], _ldw(wob)).astype(BF16)
            ostage[rows, D:640] = rb[:, 64:128]
            ostage[rows, 640:2 * D] = rb[:, 128:DP]
            oat = _dot(_ldw(mt), _pad_rows(pqs[:, o:o + t]))
            ostage[rows, 0:D] = oat.T.astype(BF16)
            c = out_copy(len(copies), starts[i] + o, t)
            copies.append(c)
            c.start()

    nb = len(BLOCKS)
    starts = [sum(BLOCKS[:i]) for i in range(nb)]
    Q = (q0, q1)
    for c in (c_xb0, c_waq, c_wob, c_wav, c_woa, c_xb1):
        c.wait()
    proj_b(0, BLOCKS[0], Q[0])
    transpose_chunks(wa_s, ua, range(0, 4))
    perm_rows(ua, 0, wq, lambda d: H * d)
    halo_first(Q[0])
    m_chain()
    prep_wob()
    carry = None
    for i in range(nb):
        p = i % 2
        if carry is not None:
            out_block(i - 1, *carry)
        if i + 1 < nb:
            halo_next(Q[p], BLOCKS[i], Q[1 - p])
            proj_b(starts[i + 1], BLOCKS[i + 1], Q[1 - p])
        carry = (a_q(starts[i], BLOCKS[i]), attn(i == 0, BLOCKS[i], Q[p]))
    out_block(nb - 1, *carry)
    for c in copies:
        c.wait()


@jax.jit
def pallas_concat_heads__linear_attn_block__sliding_local_dilated__prompt_kernel(
        A_x, A_wqkv, A_wo, B_x, B_wqkv, B_wo):
    xa = jnp.transpose(A_x, (0, 2, 1)).reshape(D, S)
    xb = jnp.transpose(B_x, (0, 2, 1)).reshape(D, S)
    hbm = pl.BlockSpec(memory_space=pl.ANY)
    out = pl.pallas_call(
        _kernel,
        out_shape=jax.ShapeDtypeStruct((S, 2 * D), BF16),
        in_specs=[hbm] * 6,
        out_specs=hbm,
        scratch_shapes=[
            pltpu.VMEM((D, S), BF16),
            pltpu.VMEM((D, S), BF16),
            pltpu.VMEM((D, 3 * D), BF16),
            pltpu.VMEM((D, 3 * D), BF16),
            pltpu.VMEM((D, D), BF16),
            pltpu.VMEM((D, D), BF16),
            pltpu.VMEM((5, D // 2 + 24, 128), U32),
            pltpu.VMEM((5, 864 + 24, 128), U32),
            pltpu.VMEM((5, D // 2 + 24, 128), U32),
            pltpu.VMEM((5, D // 2, 128), U32),
            pltpu.VMEM((5, D // 2, 128), U32),
            pltpu.VMEM((5, 896, 128), U32),
            pltpu.VMEM((5, DP // 2, 128), U32),
            pltpu.VMEM((5, D // 2, 128), U32),
            pltpu.VMEM((5, D + 24, 128), F32),
            pltpu.VMEM((D + 24, 128), F32),
            pltpu.VMEM((D, 128), F32),
            pltpu.VMEM((15, HALO + TMAX, 128), F32),
            pltpu.VMEM((15, HALO + TMAX, 128), F32),
            pltpu.VMEM((S, 2 * D), BF16),
            pltpu.SemaphoreType.DMA((11,)),
            pltpu.SemaphoreType.DMA((len(BLOCKS) + len(LAST) - 1,)),
        ],
        compiler_params=pltpu.CompilerParams(
            vmem_limit_bytes=110 * 1024 * 1024,
            flags={"XLA_TPU_EVENLY_DISTRIBUTE_CRITICAL_NODES": True}),
    )(xa, A_wqkv, A_wo, xb, B_wqkv, B_wo)
    return out.reshape(1, S, 2 * D)
```
